```python
import os as _os
_os.environ.setdefault("JAX_PLATFORMS", "cpu")
import jax
import jax.numpy as jnp

def _softmax(x, axis=-1):
    return jax.nn.softmax(x, axis=axis)
def _gelu(x):
    return jax.nn.gelu(x, approximate=True)
def _silu(x):
    return jax.nn.silu(x)
def _sigmoid(x):
    return jax.nn.sigmoid(x)
def _layernorm(x, axis=-1, eps=1e-5):
    m = jnp.mean(x, axis=axis, keepdims=True)
    v = jnp.var(x, axis=axis, keepdims=True)
    return (x - m) / jnp.sqrt(v + eps)
def _scatter_add(tgt, idx, src, axis=0):
    return tgt.at[idx].add(src)
def _segment_sum(src, seg, n):
    return jax.ops.segment_sum(src, seg, n)
class _Rng:
    def __init__(self, key):
        self._k = key
    def _next(self):
        self._k, sub = jax.random.split(self._k)
        return sub
    def normal(self, shape):
        return jax.random.normal(self._next(), shape, dtype=jnp.bfloat16)
    def randint(self, lo, hi, shape):
        return jax.random.randint(self._next(), shape, lo, hi, dtype=jnp.int32)
    def uniform(self, shape, lo=0.0, hi=1.0):
        return jax.random.uniform(self._next(), shape, jnp.bfloat16, lo, hi)
    def permutation(self, n):
        return jax.random.permutation(self._next(), n)


kernel_name = 'standalone__softmax_full_bidir__sampling'

def setup_inputs():
    _rng = _Rng(jax.random.key(int.from_bytes(__import__("os").urandom(4), "little")))
    _w = (lambda a: (lambda t: t.astype(jnp.bfloat16) if jnp.issubdtype(t.dtype, jnp.floating) else t)(jnp.asarray(a)))
    B, H, Sq, Skv, Dh = 8, 32, 1, 4096, 192
    return {
        "q": _w((lambda *s: _rng.normal(s) * 0.4)(B, H, Sq, Dh)),
        "k": _w((lambda *s: _rng.normal(s) * 0.4)(B, H, Skv, Dh)),
        "v": _w((lambda *s: _rng.normal(s) * 0.05)(B, H, Skv, Dh)),
    }

def reference(q, k, v):
    scale = q.shape[-1] ** -0.5
    scores = jnp.einsum('bhqd,bhkd->bhqk', q, k) * scale
    attn = _softmax(scores, axis=-1)
    return jnp.einsum('bhqk,bhkd->bhqd', attn, v)
```

```python
import functools

import jax
import jax.numpy as jnp
from jax import lax
import jax.experimental.pallas as pl
import jax.experimental.pallas.tpu as pltpu

LANES = 128


def build(G=16, RB=1, NBUF=4, SEG=4, M=2, order="pos", checks=False, compute=True):
    def fn(q, k, v):
        B, H, SQ, D = q.shape
        S = k.shape[2]
        NH = B * H
        NRB = D // 8
        NCT = S // LANES
        NV = NCT // 2
        NSEG = NV // SEG
        NG = NH // G
        NR = NRB // RB
        L = NBUF - 1
        NC = NG * 2 * NR
        scale = D ** -0.5

        def view(x):
            x = x.reshape(NH, NCT, LANES, NRB, 8).transpose(0, 3, 1, 4, 2)
            return x.reshape(NH, NRB, NSEG, SEG, 16, LANES)

        def kernel(q_hbm, k_hbm, v_hbm, o_hbm, buf, q_vmem, qt, acc, p_ref, ot, o_vmem, sem, qsem):
            def issue_from(src, g, r, slot):
                half = G // 2
                for rb in range(RB):
                    for sg in range(NSEG):
                        for h in range(0, half, M):
                            for t in range(2):
                                hh = t * half + h
                                pltpu.make_async_copy(
                                    src.at[pl.ds(g * G + hh, M), r * RB + rb, sg],
                                    buf.at[slot, pl.ds(hh, M), rb, sg],
                                    sem.at[slot],
                                ).start(priority=t)

            def issue(c):
                g = c // (2 * NR)
                ph = (c // NR) % 2
                r = c % NR
                slot = c % NBUF
                pl.when(jnp.logical_and(ph == 0, c < NC))(lambda: issue_from(k_hbm, g, r, slot))
                pl.when(jnp.logical_and(ph == 1, c < NC))(lambda: issue_from(v_hbm, g, r, slot))

            def wait(slot):
                pltpu.make_async_copy(buf.at[slot], buf.at[slot], sem.at[slot]).wait()

            assert L <= NR
            issue_from(k_hbm, 0, 0, 0)
            qcopy = pltpu.make_async_copy(q_hbm, q_vmem, qsem)
            qcopy.start()

            def pro(c, _):
                issue_from(k_hbm, 0, c, c)

            lax.fori_loop(1, L, pro, None)
            qcopy.wait()

            for b in range(NH // LANES):
                qf = q_vmem[pl.ds(b * LANES, LANES), :].astype(jnp.float32) * scale
                qtb = qf.T
                for j in range(LANES // G):
                    sh = (LANES - j * G) % LANES
                    qt[b * (LANES // G) + j] = pltpu.roll(qtb, sh, 1) if sh else qtb

            lane = lax.broadcasted_iota(jnp.int32, (8, LANES), 1)

            def group(g, _):
                def kstep(r, _):
                    c = g * 2 * NR + r
                    slot = c % NBUF
                    wait(slot)
                    issue(c + L)
                    if not compute:
                        return
                    row = pl.multiple_of(r * (8 * RB), 8)
                    qs = [qt[g, pl.ds(row + 8 * rb, 8), :] for rb in range(RB)]
                    first = r == 0
                    for h in range(G):
                        qb = [jnp.broadcast_to(x[:, h:h + 1], (8, LANES)) for x in qs]
                        for j in range(NV):
                            lo = hi = None
                            for rb in range(RB):
                                x = buf[slot, h, rb, j // SEG, j % SEG].astype(jnp.float32)
                                a, b = x[:8] * qb[rb], x[8:] * qb[rb]
                                lo = a if lo is None else lo + a
                                hi = b if hi is None else hi + b
                            acc[h, 2 * j] += lo
                            acc[h, 2 * j + 1] += hi

                acc[...] = jnp.zeros_like(acc)
                lax.fori_loop(0, NR, kstep, None)

                if compute:
                    for h in range(G):
                        s = jnp.sum(acc[h], axis=1)
                        m = jnp.max(s, keepdims=True)
                        e = jnp.exp(s - m)
                        p_ref[h] = e / jnp.sum(e, keepdims=True)

                def vstep(r, _):
                    c = g * 2 * NR + NR + r
                    slot = c % NBUF
                    wait(slot)
                    issue(c + L)
                    if not compute:
                        return
                    lane0 = (g * G) % LANES
                    blk = (g * G) // LANES
                    row = pl.multiple_of(r * (8 * RB), 8)
                    outs = [ot[blk, pl.ds(row + 8 * rb, 8), :] for rb in range(RB)]
                    for h in range(G):
                        a = [[None, None] for _ in range(RB)]
                        for j in range(NV):
                            p0 = jnp.broadcast_to(p_ref[h, pl.ds(2 * j, 1), :], (8, LANES))
                            p1 = jnp.broadcast_to(p_ref[h, pl.ds(2 * j + 1, 1), :], (8, LANES))
                            for rb in range(RB):
                                x = buf[slot, h, rb, j // SEG, j % SEG].astype(jnp.float32)
                                u, w = x[:8] * p0, x[8:] * p1
                                a[rb][0] = u if j == 0 else a[rb][0] + u
                                a[rb][1] = w if j == 0 else a[rb][1] + w
                        for rb in range(RB):
                            red = jnp.sum(a[rb][0] + a[rb][1], axis=1, keepdims=True)
                            outs[rb] = jnp.where(lane == lane0 + h, red, outs[rb])
                    for rb in range(RB):
                        ot[blk, pl.ds(row + 8 * rb, 8), :] = outs[rb]

                lax.fori_loop(0, NR, vstep, None)

            ot[...] = jnp.zeros_like(ot)
            lax.fori_loop(0, NG, group, None)
            for b in range(NH // LANES):
                o_vmem[pl.ds(b * LANES, LANES), :] = ot[b].T.astype(o_vmem.dtype)
            ocopy = pltpu.make_async_copy(o_vmem, o_hbm, qsem)
            ocopy.start()
            ocopy.wait()

        any_spec = pl.BlockSpec(memory_space=pl.ANY)
        out = pl.pallas_call(
            kernel,
            in_specs=[any_spec, any_spec, any_spec],
            out_specs=any_spec,
            out_shape=jax.ShapeDtypeStruct((NH, D), q.dtype),
            scratch_shapes=[
                pltpu.VMEM((NBUF, G, RB, NSEG, SEG, 16, LANES), k.dtype),
                pltpu.VMEM((NH, D), q.dtype),
                pltpu.VMEM((NG, D, LANES), jnp.float32),
                pltpu.VMEM((G, NCT, 8, LANES), jnp.float32),
                pltpu.VMEM((G, NCT, LANES), jnp.float32),
                pltpu.VMEM((NH // LANES, D, LANES), jnp.float32),
                pltpu.VMEM((NH, D), q.dtype),
                pltpu.SemaphoreType.DMA((NBUF,)),
                pltpu.SemaphoreType.DMA,
            ],
            compiler_params=pltpu.CompilerParams(
                vmem_limit_bytes=100 * 1024 * 1024, disable_bounds_checks=not checks
            ),
            name="decode_attn",
        )(q.reshape(NH, D), view(k), view(v))
        return out.reshape(B, H, SQ, D)

    return fn


@jax.jit
def pallas_standalone__softmax_full_bidir__sampling_kernel(q, k, v):
    return build(NBUF=8)(q, k, v)
```

```python
import functools

import jax
import jax.numpy as jnp
from jax import lax
import jax.experimental.pallas as pl
import jax.experimental.pallas.tpu as pltpu

LANES = 128


def _unpack(x):
    w = pltpu.bitcast(x, jnp.uint32)
    lo = pltpu.bitcast(w << 16, jnp.float32)
    hi = pltpu.bitcast(w & jnp.uint32(0xFFFF0000), jnp.float32)
    return lo, hi


def build(G=16, NBUF=4, shift=1, desc=True, checks=False, compute=True, late_issue=False, split="half"):
    def fn(q, k, v):
        B, H, SQ, D = q.shape
        S = k.shape[2]
        NH = B * H
        NRB = D // 8
        NCT = S // LANES
        PV = NCT // 4
        NP = 2 * NRB
        NG = NH // G
        L = NBUF - 1
        NC = NG * 2 * NRB
        NSLAB = NH // LANES
        scale = D ** -0.5

        def view(x):
            x = x.reshape(NH, NCT, LANES, NRB, 8).transpose(0, 3, 1, 4, 2)
            return x.reshape(NH, NP, PV, 16, LANES)

        def kernel(q_hbm, k_hbm, v_hbm, o_hbm, buf, q_vmem, qt, qd, acc, pe, ot, ot2, o_vmem, sem, qsem):
            def pieces(r):
                if shift:
                    return jnp.where(r == 0, NP - 1, 2 * r - 1), 2 * r
                return 2 * r, 2 * r + 1

            def issue_from(src, g, r, slot):
                pa, pb = pieces(r)
                half = G // 2
                hs = range(half - 1, -1, -1) if desc else range(half)
                for h in hs:
                    for j, p in enumerate((pa, pb)):
                        for t in range(2):
                            hh = t * half + h if split == "half" else 2 * h + t
                            pltpu.make_async_copy(
                                src.at[g * G + hh, p], buf.at[slot, hh, j], sem.at[slot]
                            ).start(priority=t)

            def issue(g, c):
                nxt = c >= 2 * NRB
                g2 = jnp.where(nxt, g + 1, g)
                c2 = jnp.where(nxt, c - 2 * NRB, c)
                isv = c2 >= NRB
                r = jnp.where(isv, c2 - NRB, c2)
                slot = lax.rem(c, NBUF)
                pl.when(jnp.logical_and(jnp.logical_not(isv), g2 < NG))(lambda: issue_from(k_hbm, g2, r, slot))
                pl.when(isv)(lambda: issue_from(v_hbm, g2, r, slot))

            def wait(slot):
                pltpu.make_async_copy(buf.at[slot], buf.at[slot], sem.at[slot]).wait()

            assert L <= NRB and (2 * NRB) % NBUF == 0
            issue_from(k_hbm, 0, 0, 0)
            qcopy = pltpu.make_async_copy(q_hbm, q_vmem, qsem)
            qcopy.start()

            def pro(c, _):
                issue_from(k_hbm, 0, c, c)

            lax.fori_loop(1, L, pro, None)
            acc[...] = jnp.zeros_like(acc)
            ot[...] = jnp.zeros_like(ot)
            qcopy.wait()

            for b in range(NSLAB):
                qf = q_vmem[pl.ds(b * LANES, LANES), :].astype(jnp.float32) * scale
                qt[...] = qf.T
                for u in range(4):
                    for par in range(2):
                        x = qt[pl.ds(2 * u + par, NRB, stride=8), :]
                        qd[par, b, pl.ds(u, NRB, stride=8), :] = x
                        qd[par, b, pl.ds(u + 4, NRB, stride=8), :] = x

            lane = lax.broadcasted_iota(jnp.int32, (8, LANES), 1)
            low = lax.broadcasted_iota(jnp.int32, (8, LANES), 0) < 4

            def group(g, _):
                slab = lax.div(g * G, LANES)
                lane0 = lax.rem(g * G, LANES)

                def where(r):
                    out = []
                    for j, p in enumerate(pieces(r)):
                        upper = (1 - j) if shift else j
                        out.append((pl.multiple_of(lax.div(p, 2) * 8, 8), upper * PV * 8))
                    return out

                def kstep(r, _):
                    slot = lax.rem(r, NBUF)
                    wait(slot)
                    if not late_issue:
                        issue(g, r + L)
                    if compute:
                        for j, (row, a0) in enumerate(where(r)):
                            qs = [
                                pltpu.roll(qd[par, slab, pl.ds(row, 8), :], lax.rem(LANES - lane0, LANES), 1)
                                for par in range(2)
                            ]
                            for h in range(G):
                                ql, qh = [jnp.broadcast_to(x[:, h:h + 1], (8, LANES)) for x in qs]
                                for i in range(PV):
                                    lo, hi = _unpack(buf[slot, h, j, i])
                                    acc[h, pl.ds(a0 + 8 * i, 8), :] += lo * ql + hi * qh
                    if late_issue:
                        issue(g, r + L)

                lax.fori_loop(0, NRB, kstep, None)

                if compute:
                    s = acc[:, pl.ds(0, NCT, stride=4), :]
                    for u in range(1, 4):
                        s = s + acc[:, pl.ds(u, NCT, stride=4), :]
                    acc[...] = jnp.zeros_like(acc)
                    m = jnp.max(jnp.max(s, axis=1, keepdims=True), axis=2, keepdims=True)
                    e = jnp.exp(s - m)
                    l = jnp.sum(jnp.sum(e, axis=1, keepdims=True), axis=2, keepdims=True)
                    p = e * (1.0 / l)
                    for u in range(4):
                        pe[:, pl.ds(u, NCT, stride=4), :] = p

                def vstep(r, _):
                    slot = lax.rem(NRB + r, NBUF)
                    wait(slot)
                    if not late_issue:
                        issue(g, NRB + r + L)
                    if compute:
                        for j, (row, a0) in enumerate(where(r)):
                            o = jnp.zeros((8, LANES), jnp.float32)
                            for h in range(G):
                                for i in range(PV):
                                    lo, hi = _unpack(buf[slot, h, j, i])
                                    pp = pe[h, pl.ds(a0 + 8 * i, 8), :]
                                    al = lo * pp if i == 0 else al + lo * pp
                                    ah = hi * pp if i == 0 else ah + hi * pp
                                t = jnp.where(low, al, ah) + pltpu.roll(jnp.where(low, ah, al), 4, 0)
                                o = jnp.where(lane == lane0 + h, jnp.sum(t, axis=1, keepdims=True), o)
                            ot[slab, pl.ds(row, 8), :] += o
                    if late_issue:
                        issue(g, NRB + r + L)

                lax.fori_loop(0, NRB, vstep, None)

            lax.fori_loop(0, NG, group, None)
            for b in range(NSLAB):
                for u in range(4):
                    for par in range(2):
                        ot2[pl.ds(2 * u + par, NRB, stride=8), :] = ot[b, pl.ds(u + 4 * par, NRB, stride=8), :]
                o_vmem[pl.ds(b * LANES, LANES), :] = ot2[...].T.astype(o_vmem.dtype)
            ocopy = pltpu.make_async_copy(o_vmem, o_hbm, qsem)
            ocopy.start()
            ocopy.wait()

        any_spec = pl.BlockSpec(memory_space=pl.ANY)
        out = pl.pallas_call(
            kernel,
            in_specs=[any_spec, any_spec, any_spec],
            out_specs=any_spec,
            out_shape=jax.ShapeDtypeStruct((NH, D), q.dtype),
            scratch_shapes=[
                pltpu.VMEM((NBUF, G, 2, PV, 16, LANES), k.dtype),
                pltpu.VMEM((NH, D), q.dtype),
                pltpu.VMEM((D, LANES), jnp.float32),
                pltpu.VMEM((2, NSLAB, D, LANES), jnp.float32),
                pltpu.VMEM((G, 4 * NCT, LANES), jnp.float32),
                pltpu.VMEM((G, 4 * NCT, LANES), jnp.float32),
                pltpu.VMEM((NSLAB, D, LANES), jnp.float32),
                pltpu.VMEM((D, LANES), jnp.float32),
                pltpu.VMEM((NH, D), q.dtype),
                pltpu.SemaphoreType.DMA((NBUF,)),
                pltpu.SemaphoreType.DMA,
            ],
            compiler_params=pltpu.CompilerParams(
                vmem_limit_bytes=100 * 1024 * 1024, disable_bounds_checks=not checks
            ),
            name="decode_attn",
        )(q.reshape(NH, D), view(k), view(v))
        return out.reshape(B, H, SQ, D)

    return fn


@jax.jit
def pallas_standalone__softmax_full_bidir__sampling_kernel(q, k, v):
    return build(G=8, NBUF=6)(q, k, v)
```

```python
import jax
import jax.numpy as jnp
from jax import lax
import jax.experimental.pallas as pl
import jax.experimental.pallas.tpu as pltpu

LANES = 128
SUB = 8
HEADS = 8
SLOTS = 8
STAGES = (2, 1, 1)


@jax.jit
def pallas_standalone__softmax_full_bidir__sampling_kernel(
    q: jax.Array,
    k: jax.Array,
    v: jax.Array,
):
    batch, heads, q_len, dim = q.shape
    seq = k.shape[2]
    num_heads = batch * heads
    groups = num_heads // HEADS
    pairs = HEADS // 2
    steps = dim // SUB
    tiles = seq // LANES
    half = tiles // 2
    vregs = half // 2
    ahead = SLOTS - 1
    scale = dim ** -0.5
    assert q_len == 1 and num_heads % HEADS == 0 and groups > 1
    assert dim % SUB == 0 and seq % (4 * LANES) == 0
    assert ahead <= steps and (2 * steps) % SLOTS == 0 and sum(STAGES) == pairs

    stage_lo = [pairs - sum(STAGES[: n + 1]) for n in range(len(STAGES))]
    stage_pairs = [
        list(reversed(range(lo, lo + size))) for lo, size in zip(stage_lo, STAGES)
    ]

    def view(x):
        x = x.reshape(num_heads, tiles, LANES, steps, SUB).transpose(0, 3, 1, 4, 2)
        return x.reshape(num_heads, 2 * steps, vregs, 2 * SUB, LANES)

    def kernel(q_hbm, k_hbm, v_hbm, o_hbm,
               ring, q_vmem, q_cols, score_acc, prob, out_cols, o_vmem,
               ring_sem, io_sem):
        def pieces(r):
            return jnp.where(r == 0, 2 * steps - 1, 2 * r - 1), 2 * r

        def piece_rows(r):
            return [pl.ds(pl.multiple_of(lax.div(p, 2) * SUB, SUB), SUB) for p in pieces(r)]

        def first_tile(j, u):
            return (1 - j) * half + 2 * u

        def fetch(src, g, r, slot):
            for n, stage in enumerate(stage_pairs):
                for i in stage:
                    for j, p in enumerate(pieces(r)):
                        for queue in range(2):
                            pltpu.make_async_copy(
                                src.at[g * HEADS + queue * pairs + i, p],
                                ring.at[slot, i, queue, j],
                                ring_sem.at[slot, n],
                            ).start(priority=queue)

        def wait(slot, n):
            filled = ring.at[slot, pl.ds(stage_lo[n], STAGES[n])]
            pltpu.make_async_copy(filled, filled, ring_sem.at[slot, n]).wait()

        def store_earlier_groups():
            done = pl.ds(0, groups - 1)
            return pltpu.make_async_copy(o_vmem.at[done], o_hbm.at[done], io_sem.at[1])

        def clear_scores(h):
            score_acc[h] = jnp.zeros(score_acc.shape[1:], score_acc.dtype)

        fetch(k_hbm, 0, 0, 0)
        load_q = pltpu.make_async_copy(q_hbm, q_vmem, io_sem.at[0])
        load_q.start()
        lax.fori_loop(1, ahead, lambda r, _: fetch(k_hbm, 0, r, r), None)
        lax.fori_loop(0, HEADS, lambda h, _: clear_scores(h), None)
        load_q.wait()
        lane = lax.broadcasted_iota(jnp.int32, (SUB, LANES), 1)

        def group(g, _):
            q_cols[...] = (q_vmem[g].astype(jnp.float32) * scale).T

            def k_step(r, _):
                slot = lax.rem(r, SLOTS)
                for n in range(len(STAGES)):
                    wait(slot, n)
                nxt = r + ahead
                free = lax.rem(nxt, SLOTS)
                pl.when(nxt < steps)(lambda: fetch(k_hbm, g, nxt, free))
                pl.when(nxt >= steps)(lambda: fetch(v_hbm, g, nxt - steps, free))
                for j, rows in enumerate(piece_rows(r)):
                    q_rows = q_cols[rows, :]
                    for h in range(HEADS):
                        q_h = jnp.broadcast_to(q_rows[:, h:h + 1], (SUB, LANES))
                        for u in range(vregs):
                            x = ring[slot, h % pairs, h // pairs, j, u].astype(jnp.float32)
                            t = first_tile(j, u)
                            score_acc[h, t] += x[:SUB] * q_h
                            score_acc[h, t + 1] += x[SUB:] * q_h

            lax.fori_loop(0, steps, k_step, None)

            def finish_scores(h, _):
                for t in range(tiles):
                    prob[h, pl.ds(t, 1), :] = jnp.sum(score_acc[h, t], axis=0, keepdims=True)
                clear_scores(h)

            lax.fori_loop(0, HEADS, finish_scores, None)
            s = prob[...]
            m = jnp.max(jnp.max(s, axis=1, keepdims=True), axis=2, keepdims=True)
            e = jnp.exp(s - m)
            total = jnp.sum(jnp.sum(e, axis=1, keepdims=True), axis=2, keepdims=True)
            prob[...] = e * (1.0 / total)
            out_cols[...] = jnp.zeros_like(out_cols)

            def v_step(r, _):
                slot = lax.rem(steps + r, SLOTS)
                wait(slot, 0)
                nxt = r + ahead
                free = lax.rem(steps + nxt, SLOTS)
                pl.when(nxt < steps)(lambda: fetch(v_hbm, g, nxt, free))
                pl.when(jnp.logical_and(nxt >= steps, g + 1 < groups))(
                    lambda: fetch(k_hbm, g + 1, nxt - steps, free))
                pl.when(jnp.logical_and(r == steps - 1, g == groups - 1))(
                    lambda: store_earlier_groups().start())
                partial = ([], [])
                for n, stage in enumerate(stage_pairs):
                    if n:
                        wait(slot, n)
                    for i in stage:
                        for queue in range(2):
                            h = queue * pairs + i
                            for j in range(2):
                                for u in range(vregs):
                                    x = ring[slot, i, queue, j, u].astype(jnp.float32)
                                    t = first_tile(j, u)
                                    top = x[:SUB] * prob[h, pl.ds(t, 1), :]
                                    bottom = x[SUB:] * prob[h, pl.ds(t + 1, 1), :]
                                    a, b = (top, bottom) if u == 0 else (a + top, b + bottom)
                                partial[j].append((h, a + b))
                for j, rows in enumerate(piece_rows(r)):
                    o = jnp.zeros((SUB, LANES), jnp.float32)
                    for h, y in partial[j]:
                        o = jnp.where(lane == h, jnp.sum(y, axis=1, keepdims=True), o)
                    out_cols[rows, :] += o

            lax.fori_loop(0, steps, v_step, None)
            o_vmem[g] = out_cols[:, :HEADS].T.astype(o_vmem.dtype)

        lax.fori_loop(0, groups, group, None)
        store_last_group = pltpu.make_async_copy(
            o_vmem.at[groups - 1], o_hbm.at[groups - 1], io_sem.at[0])
        store_last_group.start()
        store_earlier_groups().wait()
        store_last_group.wait()

    in_hbm = pl.BlockSpec(memory_space=pl.ANY)
    out = pl.pallas_call(
        kernel,
        in_specs=[in_hbm, in_hbm, in_hbm],
        out_specs=in_hbm,
        out_shape=jax.ShapeDtypeStruct((groups, HEADS, dim), q.dtype),
        scratch_shapes=[
            pltpu.VMEM((SLOTS, pairs, 2, 2, vregs, 2 * SUB, LANES), k.dtype),
            pltpu.VMEM((groups, HEADS, dim), q.dtype),
            pltpu.VMEM((dim, HEADS), jnp.float32),
            pltpu.VMEM((HEADS, tiles, SUB, LANES), jnp.float32),
            pltpu.VMEM((HEADS, tiles, LANES), jnp.float32),
            pltpu.VMEM((dim, LANES), jnp.float32),
            pltpu.VMEM((groups, HEADS, dim), q.dtype),
            pltpu.SemaphoreType.DMA((SLOTS, len(STAGES))),
            pltpu.SemaphoreType.DMA((2,)),
        ],
        compiler_params=pltpu.CompilerParams(
            disable_bounds_checks=True,
            disable_semaphore_checks=True,
        ),
        name="decode_attn",
    )(q.reshape(groups, HEADS, dim), view(k), view(v))
    return out.reshape(q.shape)
```
